```python
import os as _os
_os.environ.setdefault("JAX_PLATFORMS", "cpu")
import jax
import jax.numpy as jnp

def _softmax(x, axis=-1):
    return jax.nn.softmax(x, axis=axis)
def _gelu(x):
    return jax.nn.gelu(x, approximate=True)
def _silu(x):
    return jax.nn.silu(x)
def _sigmoid(x):
    return jax.nn.sigmoid(x)
def _layernorm(x, axis=-1, eps=1e-5):
    m = jnp.mean(x, axis=axis, keepdims=True)
    v = jnp.var(x, axis=axis, keepdims=True)
    return (x - m) / jnp.sqrt(v + eps)
def _scatter_add(tgt, idx, src, axis=0):
    return tgt.at[idx].add(src)
def _segment_sum(src, seg, n):
    return jax.ops.segment_sum(src, seg, n)
class _Rng:
    def __init__(self, key):
        self._k = key
    def _next(self):
        self._k, sub = jax.random.split(self._k)
        return sub
    def normal(self, shape):
        return jax.random.normal(self._next(), shape, dtype=jnp.bfloat16)
    def randint(self, lo, hi, shape):
        return jax.random.randint(self._next(), shape, lo, hi, dtype=jnp.int32)
    def uniform(self, shape, lo=0.0, hi=1.0):
        return jax.random.uniform(self._next(), shape, jnp.bfloat16, lo, hi)
    def permutation(self, n):
        return jax.random.permutation(self._next(), n)


kernel_name = 'standalone__gqa_block_cached__near_ridge'

def setup_inputs():
    _rng = _Rng(jax.random.key(int.from_bytes(__import__("os").urandom(4), "little")))
    _w = (lambda a: (lambda t: t.astype(jnp.bfloat16) if jnp.issubdtype(t.dtype, jnp.floating) else t)(jnp.asarray(a)))
    B, Sq, D = 8, 96, 640
    Hq, Hkv, Sk, Dh = 32, 32, 512, 128
    assert Hq % Hkv == 0, (Hq, Hkv)
    return {
        "x": _w((lambda *s: _rng.normal(s) * 0.2)(B, Sq, D)),
        "k_cache": _w((lambda *s: _rng.normal(s) * 3.2)(B, Hkv, Sk, Dh)),
        "v_cache": _w((lambda *s: _rng.normal(s) * 0.05)(B, Hkv, Sk, Dh)),
        "wq": _w((lambda *s: _rng.normal(s) * 0.2)(D, Hq * Dh) * (D ** -0.5)),
        "wo": _w((lambda *s: _rng.normal(s) * 0.05)(Hq * Dh, D) * ((Hq * Dh) ** -0.5)),
    }

def reference(x, k_cache, v_cache, wq, wo):
    B, Sq, D = x.shape
    Hq, Dh = 32, 128
    Hkv = k_cache.shape[1]
    rep = Hq // Hkv
    q = (lambda x, *d: x.transpose(*d))((x @ wq).reshape(B, Sq, Hq, Dh), 0, 2, 1, 3)
    k = jnp.repeat(k_cache, rep, axis=1)
    v = jnp.repeat(v_cache, rep, axis=1)
    scores = jnp.einsum("bhqd,bhkd->bhqk", q, k) * (Dh ** -0.5)
    p = _softmax(scores, axis=-1)
    o = jnp.einsum("bhqk,bhkd->bhqd", p, v)
    return (lambda x, *d: x.transpose(*d))(o, 0, 2, 1, 3).reshape(B, Sq, Hq * Dh) @ wo
```

```python
import math

import jax
import jax.numpy as jnp
import jax.experimental.pallas as pl
import jax.experimental.pallas.tpu as pltpu

_G = 8
_NS = 3


@jax.jit
def pallas_standalone__gqa_block_cached__near_ridge_kernel(
    x: jax.Array,
    k_cache: jax.Array,
    v_cache: jax.Array,
    wq: jax.Array,
    wo: jax.Array,
):
    B, Sq, D = x.shape
    Hq, Dh = 32, 128
    Hkv, Sk = k_cache.shape[1], k_cache.shape[2]
    rep = Hq // Hkv
    G, NS = _G, _NS
    assert Hq % Hkv == 0 and G % rep == 0 and Hq % G == 0
    Gk = G // rep
    NG = Hq // G
    T = NG * B
    assert NG >= 2 and T >= NS
    scale = Dh ** -0.5 * math.log2(math.e)

    def kernel(x_ref, k_hbm, v_hbm, wq_ref, wo_ref, o_ref,
               acc_scr, kbuf, vbuf, ksem, vsem):
        g = pl.program_id(0)
        b = pl.program_id(1)
        t = g * B + b

        def copies(step, slot):
            gs = step // B
            bs = step % B
            kc = pltpu.make_async_copy(
                k_hbm.at[bs, pl.ds(gs * Gk, Gk)], kbuf.at[slot], ksem.at[slot])
            vc = pltpu.make_async_copy(
                v_hbm.at[bs, pl.ds(gs * Gk, Gk)], vbuf.at[slot], vsem.at[slot])
            return kc, vc

        @pl.when(t == 0)
        def _():
            for s in range(NS - 1):
                kc, vc = copies(s, s)
                kc.start()
                vc.start()

        nxt = t + NS - 1

        @pl.when(nxt < T)
        def _():
            kc, vc = copies(nxt, nxt % NS)
            kc.start()
            vc.start()

        slot = t % NS
        kc, vc = copies(t, slot)
        kc.wait()
        vc.wait()

        q = jnp.dot(x_ref[b], wq_ref[...], preferred_element_type=jnp.float32)
        q = (q * scale).astype(jnp.bfloat16)

        def qk(h):
            qh = q[:, h * Dh:(h + 1) * Dh]
            kh = kbuf[slot, h // rep]
            return jax.lax.dot_general(qh, kh, (((1,), (1,)), ((), ())),
                                       preferred_element_type=jnp.float32)

        def rest(h, s):
            vh = vbuf[slot, h // rep]
            m = jnp.max(s, axis=-1, keepdims=True)
            p = jnp.exp2(s - m)
            l = jnp.sum(p, axis=-1, keepdims=True)
            o = jnp.dot(p.astype(jnp.bfloat16), vh,
                        preferred_element_type=jnp.float32)
            o = o / l
            return o.astype(jnp.bfloat16)

        ss = [qk(h) for h in range(G)]
        os_ = [rest(h, ss[h]) for h in range(G)]
        o_all = jnp.concatenate(os_, axis=-1)
        c = jnp.dot(o_all, wo_ref[...], preferred_element_type=jnp.float32)

        @pl.when(g == 0)
        def _():
            acc_scr[b] = c

        @pl.when(jnp.logical_and(g > 0, g < NG - 1))
        def _():
            acc_scr[b] += c

        @pl.when(g == NG - 1)
        def _():
            o_ref[0] = (acc_scr[b] + c).astype(o_ref.dtype)

    return pl.pallas_call(
        kernel,
        grid=(NG, B),
        in_specs=[
            pl.BlockSpec((B, Sq, D), lambda g, b: (0, 0, 0)),
            pl.BlockSpec(memory_space=pl.ANY),
            pl.BlockSpec(memory_space=pl.ANY),
            pl.BlockSpec((D, G * Dh), lambda g, b: (0, g)),
            pl.BlockSpec((G * Dh, D), lambda g, b: (g, 0)),
        ],
        out_specs=pl.BlockSpec(
            (1, Sq, D), lambda g, b: (jnp.where(g == NG - 1, b, 0), 0, 0)),
        out_shape=jax.ShapeDtypeStruct((B, Sq, D), x.dtype),
        scratch_shapes=[
            pltpu.VMEM((B, Sq, D), jnp.float32),
            pltpu.VMEM((NS, Gk, Sk, Dh), k_cache.dtype),
            pltpu.VMEM((NS, Gk, Sk, Dh), v_cache.dtype),
            pltpu.SemaphoreType.DMA((NS,)),
            pltpu.SemaphoreType.DMA((NS,)),
        ],
        compiler_params=pltpu.CompilerParams(
            dimension_semantics=("arbitrary", "arbitrary"),
            vmem_limit_bytes=100 * 1024 * 1024,
        ),
    )(x, k_cache, v_cache, wq, wo)
```

```python
import math

import jax
import jax.numpy as jnp
import jax.experimental.pallas as pl
import jax.experimental.pallas.tpu as pltpu

_G = 4
_NS = 4


@jax.jit
def pallas_standalone__gqa_block_cached__near_ridge_kernel(
    x: jax.Array,
    k_cache: jax.Array,
    v_cache: jax.Array,
    wq: jax.Array,
    wo: jax.Array,
):
    B, Sq, D = x.shape
    Hq, Dh = 32, 128
    Hkv, Sk = k_cache.shape[1], k_cache.shape[2]
    rep = Hq // Hkv
    G, NS = _G, _NS
    assert Hq % Hkv == 0 and G % rep == 0 and Hq % G == 0
    Gk = G // rep
    NG = Hq // G
    T = NG * B
    GD = G * Dh
    assert NG >= 2 and B >= 3 and T > NS
    scale = Dh ** -0.5 * math.log2(math.e)


    def kernel(x_hbm, k_hbm, v_hbm, wq_hbm, wo_hbm, o_hbm,
               acc_scr, q_scr, o_scr, obuf, xbuf, wqbuf, wobuf, kbuf, vbuf,
               ksem, vsem, osem, xsem, wqsem, wosem):
        g = pl.program_id(0)
        b = pl.program_id(1)
        t = g * B + b

        def kv_copies(step, slot):
            gs = step // B
            bs = step % B
            kc = pltpu.make_async_copy(
                k_hbm.at[bs, pl.ds(gs * Gk, Gk)], kbuf.at[slot], ksem.at[slot])
            vc = pltpu.make_async_copy(
                v_hbm.at[bs, pl.ds(gs * Gk, Gk)], vbuf.at[slot], vsem.at[slot])
            return kc, vc

        def wq_copy(gg):
            s = gg % 2
            return pltpu.make_async_copy(
                wq_hbm.at[:, pl.ds(pl.multiple_of(gg * GD, GD), GD)], wqbuf.at[s], wqsem.at[s])

        def wo_copy(gg):
            s = gg % 2
            return pltpu.make_async_copy(
                wo_hbm.at[pl.ds(pl.multiple_of(gg * GD, GD), GD), :], wobuf.at[s], wosem.at[s])

        def x_copy():
            return pltpu.make_async_copy(x_hbm, xbuf, xsem.at[0])

        def out_copy(bb):
            return pltpu.make_async_copy(obuf.at[bb], o_hbm.at[bb], osem.at[bb])

        def qproj(bb, ws, h):
            qh = jnp.dot(xbuf[bb], wqbuf[ws, :, h * Dh:(h + 1) * Dh],
                         preferred_element_type=jnp.float32)
            return (qh * scale).astype(jnp.bfloat16)

        @pl.when(t == 0)
        def _():
            x_copy().start()
            wq_copy(0).start()
            for s in range(NS - 1):
                kc, vc = kv_copies(s, s)
                kc.start()
                vc.start()
                if s == 0:
                    wo_copy(0).start()
            acc_scr[...] = jnp.zeros(acc_scr.shape, acc_scr.dtype)
            o_scr[1] = jnp.zeros(o_scr.shape[1:], o_scr.dtype)
            wobuf[1] = jnp.zeros(wobuf.shape[1:], wobuf.dtype)
            x_copy().wait()
            wq_copy(0).wait()
            for h in range(G):
                q_scr[0, :, h * Dh:(h + 1) * Dh] = qproj(0, 0, h)

        @pl.when(jnp.logical_and(b == 1, g < NG - 1))
        def _():
            wq_copy(g + 1).start()
            wo_copy(g + 1).start()

        nxt = t + NS - 1

        @pl.when(nxt < T)
        def _():
            kc, vc = kv_copies(nxt, nxt % NS)
            kc.start()
            vc.start()

        @pl.when(b == 1)
        def _():
            wo_copy(g).wait()

        @pl.when(jnp.logical_and(b == B - 1, g < NG - 1))
        def _():
            wq_copy(g + 1).wait()

        slot = t % NS
        kc, vc = kv_copies(t, slot)
        kc.wait()
        vc.wait()

        cur = t % 2
        oth = 1 - cur
        t_next = jnp.minimum(t + 1, T - 1)
        b_next = t_next % B
        wq_s = (t_next // B) % 2
        t_prev = jnp.maximum(t - 1, 0)
        b_prev = t_prev % B
        wo_s = jnp.where(t == 0, 1, (t_prev // B) % 2)

        def qk(h):
            qh = q_scr[cur, :, h * Dh:(h + 1) * Dh]
            kh = kbuf[slot, h // rep]
            return jax.lax.dot_general(qh, kh, (((1,), (1,)), ((), ())),
                                       preferred_element_type=jnp.float32)

        def rest(h, s):
            vh = vbuf[slot, h // rep]
            m = jnp.max(s, axis=-1, keepdims=True)
            p = jnp.exp2(s - m)
            l = jnp.sum(p, axis=-1, keepdims=True)
            o = jnp.dot(p.astype(jnp.bfloat16), vh,
                        preferred_element_type=jnp.float32)
            o = o / l
            o_scr[cur, :, h * Dh:(h + 1) * Dh] = o.astype(jnp.bfloat16)

        def oproj(which, ws, h):
            return jnp.dot(o_scr[which, :, h * Dh:(h + 1) * Dh],
                           wobuf[ws, h * Dh:(h + 1) * Dh, :],
                           preferred_element_type=jnp.float32)

        c = None
        s_next = qk(0)
        for h in range(G):
            s = s_next
            if h + 1 < G:
                s_next = qk(h + 1)
            q_scr[oth, :, h * Dh:(h + 1) * Dh] = qproj(b_next, wq_s, h)
            ch = oproj(oth, wo_s, h)
            c = ch if c is None else c + ch
            rest(h, s)
        acc_scr[b_prev] += jnp.where(t > 0, c, 0.0)

        @pl.when(jnp.logical_and(g == NG - 1, b > 0))
        def _():
            obuf[b_prev] = acc_scr[b_prev].astype(obuf.dtype)
            out_copy(b_prev).start()

        @pl.when(t == T - 1)
        def _():
            cl = None
            for h in range(G):
                ch = oproj(cur, (NG - 1) % 2, h)
                cl = ch if cl is None else cl + ch
            obuf[B - 1] = (acc_scr[B - 1] + cl).astype(obuf.dtype)
            out_copy(B - 1).start()
            for bb in range(B):
                out_copy(bb).wait()

    any_spec = pl.BlockSpec(memory_space=pl.ANY)
    return pl.pallas_call(
        kernel,
        grid=(NG, B),
        in_specs=[any_spec] * 5,
        out_specs=any_spec,
        out_shape=jax.ShapeDtypeStruct((B, Sq, D), x.dtype),
        scratch_shapes=[
            pltpu.VMEM((B, Sq, D), jnp.float32),
            pltpu.VMEM((2, Sq, GD), jnp.bfloat16),
            pltpu.VMEM((2, Sq, GD), jnp.bfloat16),
            pltpu.VMEM((B, Sq, D), x.dtype),
            pltpu.VMEM((B, Sq, D), x.dtype),
            pltpu.VMEM((2, D, GD), wq.dtype),
            pltpu.VMEM((2, GD, D), wo.dtype),
            pltpu.VMEM((NS, Gk, Sk, Dh), k_cache.dtype),
            pltpu.VMEM((NS, Gk, Sk, Dh), v_cache.dtype),
            pltpu.SemaphoreType.DMA((NS,)),
            pltpu.SemaphoreType.DMA((NS,)),
            pltpu.SemaphoreType.DMA((B,)),
            pltpu.SemaphoreType.DMA((1,)),
            pltpu.SemaphoreType.DMA((2,)),
            pltpu.SemaphoreType.DMA((2,)),
        ],
        compiler_params=pltpu.CompilerParams(
            dimension_semantics=("arbitrary", "arbitrary"),
            vmem_limit_bytes=100 * 1024 * 1024,
        ),
    )(x, k_cache, v_cache, wq, wo)
```
